```python
import jax
import jax.numpy as jnp

def _softmax(x, axis=-1):
    return jax.nn.softmax(x, axis=axis)
def _gelu(x):
    return jax.nn.gelu(x, approximate=True)
def _silu(x):
    return jax.nn.silu(x)
def _sigmoid(x):
    return jax.nn.sigmoid(x)
def _layernorm(x, axis=-1, eps=1e-5):
    m = jnp.mean(x, axis=axis, keepdims=True)
    v = jnp.var(x, axis=axis, keepdims=True)
    return (x - m) / jnp.sqrt(v + eps)
def _scatter_add(tgt, idx, src, axis=0):
    return tgt.at[idx].add(src)
def _segment_sum(src, seg, n):
    return jax.ops.segment_sum(src, seg, n)
class _Rng:
    def __init__(self, key):
        self._k = key
    def _next(self):
        self._k, sub = jax.random.split(self._k)
        return sub
    def normal(self, shape):
        return jax.random.normal(self._next(), shape, dtype=jnp.bfloat16)
    def randint(self, lo, hi, shape):
        return jax.random.randint(self._next(), shape, lo, hi, dtype=jnp.int32)
    def uniform(self, shape, lo=0.0, hi=1.0):
        return jax.random.uniform(self._next(), shape, jnp.bfloat16, lo, hi)
    def permutation(self, n):
        return jax.random.permutation(self._next(), n)


kernel_name = 'standalone__groupnorm__prompt'

def setup_inputs():
    _rng = _Rng(jax.random.key(int.from_bytes(__import__("os").urandom(4), "little")))
    _w = (lambda a: (lambda t: t.astype(jnp.bfloat16) if jnp.issubdtype(t.dtype, jnp.floating) else t)(jnp.asarray(a)))
    B = 2
    G = 32
    cpg = max(1, 1024 // G)
    C = G * cpg
    H, W = 32, 2048
    return {
        "x": _w((lambda *s: _rng.normal(s) * 0.05)(B, C, H, W)),
        "g": _w((lambda *s: _rng.normal(s) * 0.05)(C) + 1.0),
        "b": _w((lambda *s: _rng.normal(s) * 0.05)(C)),
    }

def reference(x, g, b):
    G = 32
    B, C, H, W = x.shape[0], x.shape[1], x.shape[2], x.shape[3]
    xr = x.reshape(B, G, C // G, H, W)
    mu = xr.mean(axis=(2, 3, 4), keepdims=True)
    var = ((xr - mu) ** 2).mean(axis=(2, 3, 4), keepdims=True)
    xn = (xr - mu) / jnp.sqrt(var + 1e-5)
    xn = xn.reshape(B, C, H, W)
    return xn * g[None, :, None, None] + b[None, :, None, None]
```

```python
import functools

import jax
import jax.numpy as jnp
from jax import lax
import jax.experimental.pallas as pl
import jax.experimental.pallas.tpu as pltpu

NUM_GROUPS = 32
EPS = 1e-5


def _gn_kernel(g_ref, b_ref, x_ref, o_ref, *, cpg, num_groups):
    _, h, w = x_ref.shape
    n = cpg * h * w
    grp = pl.program_id(0) % num_groups

    def sum_body(c, acc):
        xc = x_ref[c].astype(jnp.float32)
        return acc + xc.reshape(h // 8, 8, w).sum(axis=0)

    s = lax.fori_loop(0, cpg, sum_body, jnp.zeros((8, w), jnp.float32))
    mu = jnp.sum(s, keepdims=True) * (1.0 / n)

    def var_body(c, acc):
        d = x_ref[c].astype(jnp.float32) - mu
        return acc + (d * d).reshape(h // 8, 8, w).sum(axis=0)

    v = lax.fori_loop(0, cpg, var_body, jnp.zeros((8, w), jnp.float32))
    var = jnp.sum(v, keepdims=True) * (1.0 / n)
    rstd = lax.rsqrt(var + EPS)

    def norm_body(c, carry):
        ch = grp * cpg + c
        scale = rstd * g_ref[ch]
        shift = b_ref[ch] - mu * scale
        o_ref[c] = (x_ref[c].astype(jnp.float32) * scale + shift).astype(o_ref.dtype)
        return carry

    lax.fori_loop(0, cpg, norm_body, 0)


@jax.jit
def pallas_standalone__groupnorm__prompt_kernel(x, g, b):
    B, C, H, W = x.shape
    G = NUM_GROUPS
    cpg = C // G
    xr = x.reshape(B * C, H, W)
    out = pl.pallas_call(
        functools.partial(_gn_kernel, cpg=cpg, num_groups=G),
        grid=(B * G,),
        in_specs=[
            pl.BlockSpec(memory_space=pltpu.SMEM),
            pl.BlockSpec(memory_space=pltpu.SMEM),
            pl.BlockSpec((cpg, H, W), lambda i: (i, 0, 0)),
        ],
        out_specs=pl.BlockSpec((cpg, H, W), lambda i: (i, 0, 0)),
        out_shape=jax.ShapeDtypeStruct(xr.shape, x.dtype),
        compiler_params=pltpu.CompilerParams(
            dimension_semantics=("arbitrary",),
            vmem_limit_bytes=64 * 1024 * 1024,
        ),
    )(g.astype(jnp.float32), b.astype(jnp.float32), xr)
    return out.reshape(B, C, H, W)
```

```python
import functools

import jax
import jax.numpy as jnp
from jax import lax
import jax.experimental.pallas as pl
import jax.experimental.pallas.tpu as pltpu

NUM_GROUPS = 32
EPS = 1e-5

TR = 8
ACC_W = 256


def _gn_kernel(g_ref, b_ref, x_hbm, o_hbm, buf, part, stat, rsem0, rsem1, wsem,
               *, rounds, blk, upg, rcols, rwin, wwin, wpre, rtail, wtail,
               rows_per_ch, units_per_batch):
    _, S, _, W = x_hbm.shape
    nh = W // rcols
    rpb = S * nh
    gpb = blk // upg
    ch_per_unit = S // rows_per_ch
    n_pos = upg * S * (W // ACC_W)
    n_acc = TR * ACC_W

    def rd_idx(i):
        bi = i // rpb
        r = i % rpb
        return bi * blk, r // nh, pl.multiple_of((r % nh) * rcols, 128)

    def rd0(base, i):
        a, s, c = rd_idx(i)
        return pltpu.make_async_copy(
            x_hbm.at[pl.ds(base + a, 1), s, :, pl.ds(c, rcols)],
            buf.at[pl.ds(a, 1), s, :, pl.ds(c, rcols)],
            rsem0.at[i % rwin])

    def rd1(base, i):
        a, s, c = rd_idx(i)
        return pltpu.make_async_copy(
            x_hbm.at[pl.ds(base + a + 1, blk - 1), s, :, pl.ds(c, rcols)],
            buf.at[pl.ds(a + 1, blk - 1), s, :, pl.ds(c, rcols)],
            rsem1.at[i % rwin])

    def rd_start(base, i):
        rd1(base, i).start(priority=1)
        rd0(base, i).start(priority=0)

    def rd_wait(base, i):
        rd0(base, i).wait()
        rd1(base, i).wait()

    def wr(base, k):
        a = (k // S) * blk
        s = k % S
        return pltpu.make_async_copy(
            buf.at[pl.ds(a, blk), s], o_hbm.at[pl.ds(base + a, blk), s],
            wsem.at[k % wwin])

    def shifts(bi):
        return tuple(
            buf[bi * blk + q * upg, 0, :, 0:ACC_W].astype(jnp.float32)
            for q in range(gpb))

    def accumulate(i, ks, acc):
        a, s, c = rd_idx(i)
        acc = list(acc)
        for u in range(blk):
            q = u // upg
            xf = buf[a + u, s, :, pl.ds(c, rcols)].astype(jnp.float32)
            s1, s2 = acc[2 * q], acc[2 * q + 1]
            for j in range(rcols // ACC_W):
                d = xf[:, j * ACC_W:(j + 1) * ACC_W] - ks[q]
                s1 = s1 + d
                s2 = s2 + d * d
            acc[2 * q], acc[2 * q + 1] = s1, s2
        return tuple(acc)

    def save_partials(bi, ks, acc):
        for q in range(gpb):
            part[bi * gpb + q, 0] = ks[q]
            part[bi * gpb + q, 1] = acc[2 * q]
            part[bi * gpb + q, 2] = acc[2 * q + 1]

    def finalize(bi):
        for q in range(gpb):
            k = part[bi * gpb + q, 0]
            s1 = part[bi * gpb + q, 1]
            s2 = part[bi * gpb + q, 2]
            d1 = s1 * (1.0 / n_pos)
            m = k + d1
            mean = jnp.sum(m, keepdims=True) * (1.0 / n_acc)
            e = m - mean
            t = (s2 - s1 * d1) * (1.0 / n_pos) + e * e
            var = jnp.maximum(jnp.sum(t, keepdims=True) * (1.0 / n_acc), 0.0)
            rstd = lax.rsqrt(var + EPS)
            stat[q, 0] = jnp.broadcast_to(mean, (TR, 128))
            stat[q, 1] = jnp.broadcast_to(rstd, (TR, 128))

    def normalize(base, k):
        a = (k // S) * blk
        s = k % S
        for u in range(blk):
            q = u // upg
            ch = ((base + a + u) % units_per_batch) * ch_per_unit + s // rows_per_ch
            scale = stat[q, 1] * g_ref[ch]
            shift = b_ref[ch] - stat[q, 0] * scale
            xf = buf[a + u, s].astype(jnp.float32)
            y = xf * jnp.tile(scale, (1, W // 128)) + jnp.tile(shift, (1, W // 128))
            buf[a + u, s] = y.astype(buf.dtype)

    zeros = tuple(jnp.zeros((TR, ACC_W), jnp.float32) for _ in range(2 * gpb))

    base = 0
    for ri, nu in enumerate(rounds):
        nblk = nu // blk
        nr = nblk * rpb
        nw = nblk * S

        if ri == 0:
            for i in range(rwin):
                rd_start(base, i)
        rd_wait(base, 0)
        rd_start(base, rwin)

        def rd_body(i, ks, acc, base=base):
            acc = accumulate(i, ks, acc)
            rd_wait(base, i + 1)
            rd_start(base, i + 1 + rwin)
            return acc

        def blk_body(bi, carry, base=base, rd_body=rd_body):
            ks = shifts(bi)
            acc = lax.fori_loop(
                0, rpb, lambda r, acc: rd_body(bi * rpb + r, ks, acc), zeros)
            save_partials(bi, ks, acc)
            return carry

        lax.fori_loop(0, nblk - 1, blk_body, 0)

        bi = nblk - 1
        ks = shifts(bi)
        n_issue = rpb - rwin - 1
        acc = lax.fori_loop(
            0, n_issue, lambda r, acc: rd_body(bi * rpb + r, ks, acc), zeros)
        finalize(0)
        for k in range(wpre):
            normalize(base, k)
        for i in range(nr - rwin - 1, nr):
            acc = accumulate(i, ks, acc)
            if i + 1 < nr:
                rd_wait(base, i + 1)
            if i + 1 == nr - 1 - rtail:
                for k in range(wpre):
                    wr(base, k).start()
        save_partials(bi, ks, acc)

        def wr_body(k, carry, base=base):
            @pl.when(k % S == 0)
            def _():
                finalize(k // S)

            normalize(base, k)

            @pl.when(k >= wwin)
            def _():
                wr(base, k - wwin).wait()

            wr(base, k).start()
            return carry

        lax.fori_loop(wpre, nw, wr_body, 0)
        for k in range(nw - wwin, nw):
            if k == nw - wtail and ri + 1 < len(rounds):
                for i in range(rwin):
                    rd_start(base + nu, i)
            wr(base, k).wait()
        if wtail == 0 and ri + 1 < len(rounds):
            for i in range(rwin):
                rd_start(base + nu, i)
        base += nu


def _groupnorm(x, g, b, *, S=32, blk=8, rcols=1024, rwin=8, wwin=8, wpre=2,
               rtail=2, wtail=1, rounds=None, max_units=88, interpret=False):
    B, C, H, W = x.shape
    G = NUM_GROUPS
    cpg = C // G
    rows_per_ch = H // TR
    assert H % TR == 0 and S % rows_per_ch == 0 and W % rcols == 0
    tr_per_group = cpg * rows_per_ch
    assert tr_per_group % S == 0
    upg = tr_per_group // S
    A = B * G * upg
    assert blk % upg == 0 and A % blk == 0
    if rounds is None:
        nblk = A // blk
        nround = -(-nblk // (max_units // blk))
        rounds = tuple(
            blk * (nblk // nround + (1 if r < nblk % nround else 0))
            for r in range(nround))
    assert sum(rounds) == A and all(r % blk == 0 and r >= 2 * blk for r in rounds)
    na = max(rounds)
    xr = x.reshape(A, S, TR, W)
    kern = functools.partial(
        _gn_kernel, rounds=rounds, blk=blk, upg=upg, rcols=rcols, rwin=rwin,
        wwin=wwin, wpre=wpre, rtail=rtail, wtail=wtail,
        rows_per_ch=rows_per_ch, units_per_batch=G * upg)
    buf_bytes = na * S * TR * W * x.dtype.itemsize
    out = pl.pallas_call(
        kern,
        in_specs=[
            pl.BlockSpec(memory_space=pltpu.SMEM),
            pl.BlockSpec(memory_space=pltpu.SMEM),
            pl.BlockSpec(memory_space=pl.ANY),
        ],
        out_specs=pl.BlockSpec(memory_space=pl.ANY),
        out_shape=jax.ShapeDtypeStruct(xr.shape, x.dtype),
        scratch_shapes=[
            pltpu.VMEM((na, S, TR, W), x.dtype),
            pltpu.VMEM((na // upg, 3, TR, ACC_W), jnp.float32),
            pltpu.VMEM((blk // upg, 2, TR, 128), jnp.float32),
            pltpu.SemaphoreType.DMA((rwin,)),
            pltpu.SemaphoreType.DMA((rwin,)),
            pltpu.SemaphoreType.DMA((wwin,)),
        ],
        compiler_params=pltpu.CompilerParams(
            vmem_limit_bytes=buf_bytes + 8 * 1024 * 1024,
        ),
        interpret=interpret,
    )(g.astype(jnp.float32), b.astype(jnp.float32), xr)
    return out.reshape(B, C, H, W)


@jax.jit
def pallas_standalone__groupnorm__prompt_kernel(x, g, b):
    return _groupnorm(x, g, b)
```

```python
import functools

import jax
import jax.numpy as jnp
from jax import lax
import jax.experimental.pallas as pl
import jax.experimental.pallas.tpu as pltpu

NUM_GROUPS = 32
EPS = 1e-5

TR = 8
LANES = 128


def _div(i, n):
    if isinstance(i, int):
        return i // n
    if n & (n - 1) == 0:
        return lax.shift_right_logical(i, n.bit_length() - 1)
    return lax.div(i, n)


def _mod(i, n):
    if isinstance(i, int):
        return i % n
    if n & (n - 1) == 0:
        return lax.bitwise_and(i, n - 1)
    return lax.rem(i, n)


def _gn_kernel(g_hbm, b_hbm, x_hbm, o_hbm,
               buf, gb, gtab, part, coef, psem, rsem, wsem,
               *, rounds, upg, rb, rcols, m0, wcols, rwin, wwin, wpre, rtail,
               wtail, rows_per_ch, accw):
    _, blk, S, _, W = x_hbm.shape
    nh = W // rcols
    rpb = S * nh
    gpb = blk // upg
    gpr = gpb * rb
    ch_per_unit = S // rows_per_ch
    cpb = blk * ch_per_unit
    cpg = upg * ch_per_unit
    n_ch = gtab.shape[1]
    n_pos = upg * S * (W // accw)
    n_acc = TR * accw
    wps = blk * S

    def rd_idx(t):
        r = _mod(t, rpb)
        c = _mod(r, nh) * rcols
        if not isinstance(c, int):
            c = pl.multiple_of(c, LANES)
        return _div(t, rpb) * rb, _div(r, nh), c

    def rd_start(base, t):
        b0, s, c = rd_idx(t)
        sem = rsem.at[_mod(t, rwin)]

        def cp(j, u0, n):
            return pltpu.make_async_copy(
                x_hbm.at[base + b0 + j, pl.ds(u0, n), s, :, pl.ds(c, rcols)],
                buf.at[b0 + j, pl.ds(u0, n), s, :, pl.ds(c, rcols)], sem)

        cp(0, m0, blk - m0).start(priority=1)
        for j in range(1, rb):
            cp(j, 0, blk).start(priority=1)
        cp(0, 0, m0).start(priority=0)

    def rd_wait(base, t):
        b0, s, c = rd_idx(t)
        pltpu.make_async_copy(
            x_hbm.at[pl.ds(base + b0, rb), :, s, :, pl.ds(c, rcols)],
            buf.at[pl.ds(b0, rb), :, s, :, pl.ds(c, rcols)],
            rsem.at[_mod(t, rwin)]).wait()

    def wr_start(base, b0, n, k, slot):
        u = _div(k, S)
        s = _mod(k, S)
        for c in range(0, W, wcols):
            pltpu.make_async_copy(
                buf.at[pl.ds(b0, n), u, s, :, pl.ds(c, wcols)],
                o_hbm.at[pl.ds(base + b0, n), u, s, :, pl.ds(c, wcols)],
                wsem.at[slot]).start()

    def wr_wait(base, b0, n, k, slot):
        u = _div(k, S)
        s = _mod(k, S)
        pltpu.make_async_copy(
            buf.at[pl.ds(b0, n), u, s], o_hbm.at[pl.ds(base + b0, n), u, s],
            wsem.at[slot]).wait()

    def shifts(b0):
        return tuple(
            buf[b0 + q // gpb, (q % gpb) * upg, 0, :, 0:accw].astype(jnp.float32)
            for q in range(gpr))

    def accumulate(t, ks, acc):
        b0, s, c = rd_idx(t)
        acc = list(acc)
        for j in range(rb):
            for u in range(blk):
                q = j * gpb + u // upg
                xf = buf[b0 + j, u, s, :, pl.ds(c, rcols)].astype(jnp.float32)
                s1, s2 = acc[2 * q], acc[2 * q + 1]
                for i in range(rcols // accw):
                    d = xf[:, i * accw:(i + 1) * accw] - ks[q]
                    s1 = s1 + d
                    s2 = s2 + d * d
                acc[2 * q], acc[2 * q + 1] = s1, s2
        return tuple(acc)

    def save_partials(b0, ks, acc):
        for q in range(gpr):
            part[0, b0 * gpb + q] = ks[q]
            part[1, b0 * gpb + q] = acc[2 * q]
            part[2, b0 * gpb + q] = acc[2 * q + 1]

    def finalize(base, b0, nb):
        g0, ng = b0 * gpb, nb * gpb
        k = part[0, g0:g0 + ng]
        s1 = part[1, g0:g0 + ng]
        s2 = part[2, g0:g0 + ng]
        d1 = s1 * (1.0 / n_pos)
        m = k + d1
        mean = jnp.sum(m, axis=(1, 2), keepdims=True) * (1.0 / n_acc)
        e = m - mean
        t = (s2 - s1 * d1) * (1.0 / n_pos) + e * e
        var = jnp.sum(t, axis=(1, 2), keepdims=True) * (1.0 / n_acc)
        rstd = lax.rsqrt(jnp.maximum(var, 0.0) + EPS)
        for i in range(ng):
            ch0 = ((base + b0) * gpb + i) * cpg % n_ch
            scale = gtab[0, ch0:ch0 + cpg] * rstd[i]
            r0 = (g0 + i) * cpg
            coef[0, r0:r0 + cpg] = scale
            coef[1, r0:r0 + cpg] = gtab[1, ch0:ch0 + cpg] - mean[i] * scale

    def normalize(b0, n, k):
        u = _div(k, S)
        s = _mod(k, S)
        row0 = _div(k, rows_per_ch)
        for j in range(n):
            row = row0 + (b0 + j) * cpb
            scale = jnp.broadcast_to(coef[0, pl.ds(row, 1), :], (TR, LANES))
            shift = jnp.broadcast_to(coef[1, pl.ds(row, 1), :], (TR, LANES))
            xf = buf[b0 + j, u, s].astype(jnp.float32)
            y = (xf * jnp.tile(scale, (1, W // LANES))
                 + jnp.tile(shift, (1, W // LANES)))
            buf[b0 + j, u, s] = y.astype(buf.dtype)

    def rd_prologue(base):
        for t in range(rwin):
            rd_start(base, t)

    zeros = tuple(jnp.zeros((TR, accw), jnp.float32) for _ in range(2 * gpr))

    rd_prologue(0)
    pcopies = [pltpu.make_async_copy(src, gb.at[i], psem.at[i])
               for i, src in enumerate((g_hbm, b_hbm))]
    for cp in pcopies:
        cp.start()

    def build_tables():
        for cp in pcopies:
            cp.wait()
        for i in range(2):
            v = gb[i].astype(jnp.float32)
            for r in range(v.shape[0]):
                gtab[i, r * LANES:(r + 1) * LANES] = jnp.broadcast_to(
                    v[r:r + 1, :], (LANES, LANES)).T

    base = 0
    for ri, sets in enumerate(rounds):
        nblk = sum(sets)
        nrb = nblk // rb
        nr = nrb * rpb
        last = ri + 1 == len(rounds)

        rd_wait(base, 0)
        rd_start(base, rwin)

        def rd_body(t, ks, acc, base=base):
            acc = accumulate(t, ks, acc)
            rd_wait(base, t + 1)
            rd_start(base, t + 1 + rwin)
            return acc

        def blk_body(bi, carry, rd_body=rd_body):
            ks = shifts(bi * rb)
            acc = lax.fori_loop(
                0, rpb, lambda r, acc: rd_body(bi * rpb + r, ks, acc), zeros)
            save_partials(bi * rb, ks, acc)
            return carry

        lax.fori_loop(0, nrb - 1, blk_body, 0)
        bl = nblk - rb
        ks = shifts(bl)
        acc = lax.fori_loop(
            nr - rpb, nr - rwin - 1, lambda t, acc: rd_body(t, ks, acc), zeros)

        n0 = sets[0]
        if ri == 0:
            build_tables()
        finalize(base, 0, n0)
        for k in range(wpre):
            normalize(0, n0, k)
        for t in range(nr - rwin, nr - rtail):
            rd_wait(base, t)
        for k in range(wpre):
            wr_start(base, 0, n0, k, k)

        def wr_fill(k, carry, base=base, n0=n0):
            normalize(0, n0, k)
            wr_start(base, 0, n0, k, k)
            return carry

        lax.fori_loop(wpre, wwin, wr_fill, 0)
        for t in range(nr - rtail, nr):
            rd_wait(base, t)

        acc = lax.fori_loop(
            nr - rwin - 1, nr, lambda t, acc: accumulate(t, ks, acc), acc)
        save_partials(bl, ks, acc)
        finalize(base, n0, nblk - n0)

        b0 = 0
        for si, n in enumerate(sets):
            if si > 0:
                def wr_edge(k, carry, base=base, b0=b0, n=n, np_=sets[si - 1]):
                    normalize(b0, n, k)
                    wr_wait(base, b0 - np_, np_, wps - wwin + k, k)
                    wr_start(base, b0, n, k, k)
                    return carry

                lax.fori_loop(0, wwin, wr_edge, 0)

            def wr_body(k, carry, base=base, b0=b0, n=n):
                slot = _mod(k, wwin)
                normalize(b0, n, k)
                wr_wait(base, b0, n, k - wwin, slot)
                wr_start(base, b0, n, k, slot)
                return carry

            lax.fori_loop(wwin, wps, wr_body, 0)
            b0 += n

        n = sets[-1]
        for k in range(wps - wwin, wps + 1):
            if k == wps - wtail and not last:
                rd_prologue(base + nblk)
            if k < wps:
                wr_wait(base, nblk - n, n, k, k % wwin)
        base += nblk


def _groupnorm(x, g, b, *, S=32, blk=8, rb=2, rcols=256, m0=2, wcols=256,
               rwin=16, wwin=16, wpre=2, rtail=6, wtail=1,
               rounds=((6, 6), (5, 5), (5, 5)), accw=256,
               nochecks=True, interpret=False):
    B, C, H, W = x.shape
    G = NUM_GROUPS
    cpg = C // G
    rows_per_ch = H // TR
    assert H % TR == 0 and S % rows_per_ch == 0
    assert W % rcols == 0 and W % wcols == 0 and rcols % accw == 0
    assert C % LANES == 0
    tr_per_group = cpg * rows_per_ch
    assert tr_per_group % S == 0
    upg = tr_per_group // S
    A = B * G * upg
    assert blk % upg == 0 and A % blk == 0
    nblk = A // blk
    assert sum(sum(r) for r in rounds) == nblk
    for r in rounds:
        assert sum(r) % rb == 0 and len(r) >= 2 and r[0] <= sum(r) - rb
    assert wpre <= wwin and (blk * S) % wwin == 0
    nb = max(sum(r) for r in rounds)
    gpb = blk // upg
    xr = x.reshape(nblk, blk, S, TR, W)
    kern = functools.partial(
        _gn_kernel, rounds=rounds, upg=upg, rb=rb, rcols=rcols, m0=m0,
        wcols=wcols, rwin=rwin, wwin=wwin, wpre=wpre, rtail=rtail, wtail=wtail,
        rows_per_ch=rows_per_ch, accw=accw)
    buf_bytes = nb * blk * S * TR * W * x.dtype.itemsize
    out = pl.pallas_call(
        kern,
        in_specs=[pl.BlockSpec(memory_space=pl.ANY)] * 3,
        out_specs=pl.BlockSpec(memory_space=pl.ANY),
        out_shape=jax.ShapeDtypeStruct(xr.shape, x.dtype),
        scratch_shapes=[
            pltpu.VMEM((nb, blk, S, TR, W), x.dtype),
            pltpu.VMEM((2, C // LANES, LANES), g.dtype),
            pltpu.VMEM((2, C, LANES), jnp.float32),
            pltpu.VMEM((3, nb * gpb, TR, accw), jnp.float32),
            pltpu.VMEM((2, nb * gpb * cpg, LANES), jnp.float32),
            pltpu.SemaphoreType.DMA((2,)),
            pltpu.SemaphoreType.DMA((rwin,)),
            pltpu.SemaphoreType.DMA((wwin,)),
        ],
        compiler_params=pltpu.CompilerParams(
            vmem_limit_bytes=buf_bytes + 10 * 1024 * 1024,
            disable_bounds_checks=nochecks,
            disable_semaphore_checks=nochecks,
        ),
        interpret=interpret,
    )(g.reshape(C // LANES, LANES), b.reshape(C // LANES, LANES), xr)
    return out.reshape(B, C, H, W)


@jax.jit
def pallas_standalone__groupnorm__prompt_kernel(x, g, b):
    return _groupnorm(x, g, b)
```

```python
import functools

import jax
import jax.numpy as jnp
from jax import lax
import jax.experimental.pallas as pl
import jax.experimental.pallas.tpu as pltpu

NUM_GROUPS = 32
EPS = 1e-5

TR = 8
LANES = 128


def _div(i, n):
    if isinstance(i, int):
        return i // n
    if n & (n - 1) == 0:
        return lax.shift_right_logical(i, n.bit_length() - 1)
    return lax.div(i, n)


def _mod(i, n):
    if isinstance(i, int):
        return i % n
    if n & (n - 1) == 0:
        return lax.bitwise_and(i, n - 1)
    return lax.rem(i, n)


def _gn_kernel(g_hbm, b_hbm, x_hbm, o_hbm,
               buf, gb, gtab, part, coef, psem, rsem, wsem,
               *, rounds, upg, rb, rcols, m0, wcols, rwin, wwin, wpre, rtail,
               wtail, rows_per_ch):
    _, blk, S, _, W = x_hbm.shape
    nh = W // rcols
    rpb = S * nh
    gpb = blk // upg
    gpr = gpb * rb
    ch_per_unit = S // rows_per_ch
    cpb = blk * ch_per_unit
    cpg = upg * ch_per_unit
    n_ch = gtab.shape[1]
    n_pos = upg * rpb
    n_acc = TR * rcols
    wps = blk * S

    def rd_idx(t):
        r = _mod(t, rpb)
        c = _mod(r, nh) * rcols
        if not isinstance(c, int):
            c = pl.multiple_of(c, LANES)
        return _div(t, rpb) * rb, _div(r, nh), c

    def rd_start(base, t):
        b0, s, c = rd_idx(t)
        sem = rsem.at[_mod(t, rwin)]

        def cp(j, u0, n):
            return pltpu.make_async_copy(
                x_hbm.at[base + b0 + j, pl.ds(u0, n), s, :, pl.ds(c, rcols)],
                buf.at[b0 + j, pl.ds(u0, n), s, :, pl.ds(c, rcols)], sem)

        cp(0, m0, blk - m0).start(priority=1)
        for j in range(1, rb):
            cp(j, 0, blk).start(priority=1)
        cp(0, 0, m0).start(priority=0)

    def rd_wait(base, t):
        b0, s, c = rd_idx(t)
        pltpu.make_async_copy(
            x_hbm.at[pl.ds(base + b0, rb), :, s, :, pl.ds(c, rcols)],
            buf.at[pl.ds(b0, rb), :, s, :, pl.ds(c, rcols)],
            rsem.at[_mod(t, rwin)]).wait()

    def wr_start(base, b0, n, k, slot):
        u = _div(k, S)
        s = _mod(k, S)
        for c in range(0, W, wcols):
            pltpu.make_async_copy(
                buf.at[pl.ds(b0, n), u, s, :, pl.ds(c, wcols)],
                o_hbm.at[pl.ds(base + b0, n), u, s, :, pl.ds(c, wcols)],
                wsem.at[slot]).start()

    def wr_wait(base, b0, n, k, slot):
        u = _div(k, S)
        s = _mod(k, S)
        pltpu.make_async_copy(
            buf.at[pl.ds(b0, n), u, s], o_hbm.at[pl.ds(base + b0, n), u, s],
            wsem.at[slot]).wait()

    def rd_prologue(base):
        for t in range(rwin):
            rd_start(base, t)

    def load_chunk(t):
        b0, s, c = rd_idx(t)
        xb = buf[pl.ds(b0, rb), :, s, :, pl.ds(c, rcols)]
        return xb.astype(jnp.float32).reshape(gpr, upg, TR, rcols)

    def shifts(t):
        return load_chunk(t)[:, 0]

    def accumulate(t, ks, acc):
        d = load_chunk(t) - ks[:, None]
        return acc[0] + jnp.sum(d, axis=1), acc[1] + jnp.sum(d * d, axis=1)

    def save_partials(b0, ks, acc):
        for i, v in enumerate((ks,) + acc):
            part[i, pl.ds(b0 * gpb, gpr)] = v

    def finalize(base, b0, nb):
        g0, ng = b0 * gpb, nb * gpb
        k = part[0, g0:g0 + ng]
        s1 = part[1, g0:g0 + ng]
        s2 = part[2, g0:g0 + ng]
        d1 = s1 * (1.0 / n_pos)
        m = k + d1
        mean = jnp.sum(m, axis=(1, 2), keepdims=True) * (1.0 / n_acc)
        e = m - mean
        t = (s2 - s1 * d1) * (1.0 / n_pos) + e * e
        var = jnp.sum(t, axis=(1, 2), keepdims=True) * (1.0 / n_acc)
        rstd = lax.rsqrt(jnp.maximum(var, 0.0) + EPS)
        for i in range(ng):
            ch0 = ((base + b0) * gpb + i) * cpg % n_ch
            r0 = (g0 + i) * cpg
            coef[0, r0:r0 + cpg] = jnp.broadcast_to(mean[i], (cpg, LANES))
            coef[1, r0:r0 + cpg] = gtab[0, ch0:ch0 + cpg] * rstd[i]
            coef[2, r0:r0 + cpg] = gtab[1, ch0:ch0 + cpg]

    def normalize(b0, n, k):
        u = _div(k, S)
        s = _mod(k, S)
        row0 = _div(k, rows_per_ch)
        for j in range(n):
            cf = coef[:, pl.ds(row0 + (b0 + j) * cpb, 1), :]
            cf = jnp.tile(jnp.broadcast_to(cf, (3, TR, LANES)), (1, 1, W // LANES))
            xf = buf[b0 + j, u, s].astype(jnp.float32)
            buf[b0 + j, u, s] = ((xf - cf[0]) * cf[1] + cf[2]).astype(buf.dtype)

    zeros = (jnp.zeros((gpr, TR, rcols), jnp.float32),) * 2

    pcopies = [pltpu.make_async_copy(src, gb.at[i], psem.at[i])
               for i, src in enumerate((g_hbm, b_hbm))]
    for cp in pcopies:
        cp.start()
    rd_prologue(0)
    for cp in pcopies:
        cp.wait()
    for i in range(2):
        v = gb[i].astype(jnp.float32)
        for r in range(v.shape[0]):
            gtab[i, r * LANES:(r + 1) * LANES] = jnp.broadcast_to(
                v[r:r + 1, :], (LANES, LANES)).T

    base = 0
    for ri, sets in enumerate(rounds):
        nblk = sum(sets)
        nrb = nblk // rb
        nr = nrb * rpb
        last = ri + 1 == len(rounds)

        rd_wait(base, 0)
        rd_start(base, rwin)

        def rd_body(t, ks, acc, base=base):
            acc = accumulate(t, ks, acc)
            rd_wait(base, t + 1)
            rd_start(base, t + 1 + rwin)
            return acc

        def blk_body(bi, carry, rd_body=rd_body):
            ks = shifts(bi * rpb)
            acc = lax.fori_loop(
                0, rpb, lambda r, acc: rd_body(bi * rpb + r, ks, acc), zeros)
            save_partials(bi * rb, ks, acc)
            return carry

        lax.fori_loop(0, nrb - 1, blk_body, 0)
        ks = shifts(nr - rpb)
        acc = lax.fori_loop(
            nr - rpb, nr - rwin - 1, lambda t, acc: rd_body(t, ks, acc), zeros)

        n0 = sets[0]
        finalize(base, 0, n0)
        for k in range(wpre):
            normalize(0, n0, k)
        for t in range(nr - rwin, nr - rtail):
            rd_wait(base, t)
        for k in range(wpre):
            wr_start(base, 0, n0, k, k)

        def wr_fill(k, carry, base=base, n0=n0):
            normalize(0, n0, k)
            wr_start(base, 0, n0, k, k)
            return carry

        lax.fori_loop(wpre, wwin, wr_fill, 0)
        for t in range(nr - rtail, nr):
            rd_wait(base, t)
        acc = lax.fori_loop(
            nr - rwin - 1, nr, lambda t, acc: accumulate(t, ks, acc), acc)
        save_partials(nblk - rb, ks, acc)
        finalize(base, n0, nblk - n0)

        b0 = 0
        for si, n in enumerate(sets):
            if si > 0:
                def wr_edge(k, carry, base=base, b0=b0, n=n, np_=sets[si - 1]):
                    normalize(b0, n, k)
                    wr_wait(base, b0 - np_, np_, wps - wwin + k, k)
                    wr_start(base, b0, n, k, k)
                    return carry

                lax.fori_loop(0, wwin, wr_edge, 0)

            def wr_body(k, carry, base=base, b0=b0, n=n):
                slot = _mod(k, wwin)
                normalize(b0, n, k)
                wr_wait(base, b0, n, k - wwin, slot)
                wr_start(base, b0, n, k, slot)
                return carry

            lax.fori_loop(wwin, wps, wr_body, 0)
            b0 += n

        n = sets[-1]
        for k in range(wps - wwin, wps + 1):
            if k == wps - wtail and not last:
                rd_prologue(base + nblk)
            if k < wps:
                wr_wait(base, nblk - n, n, k, k % wwin)
        base += nblk


def _groupnorm(x, g, b, *, S=32, blk=8, rb=2, rcols=256, m0=2, wcols=256,
               rwin=16, wwin=16, wpre=2, rtail=8, wtail=1,
               rounds=((6, 6), (5, 5), (5, 5)), interpret=False):
    B, C, H, W = x.shape
    G = NUM_GROUPS
    cpg = C // G
    rows_per_ch = H // TR
    assert H % TR == 0 and S % rows_per_ch == 0
    assert W % rcols == 0 and W % wcols == 0 and C % LANES == 0
    tr_per_group = cpg * rows_per_ch
    assert tr_per_group % S == 0
    upg = tr_per_group // S
    A = B * G * upg
    assert blk % upg == 0 and A % blk == 0
    nblk = A // blk
    assert sum(sum(r) for r in rounds) == nblk
    for r in rounds:
        assert sum(r) % rb == 0 and len(r) >= 2 and rb <= r[0] <= sum(r) - rb
    assert wpre <= wwin and (blk * S) % wwin == 0 and wtail <= wwin
    assert rtail <= rwin < S * (W // rcols) and 0 < m0 < blk
    nb = max(sum(r) for r in rounds)
    gpb = blk // upg
    xr = x.reshape(nblk, blk, S, TR, W)
    kern = functools.partial(
        _gn_kernel, rounds=rounds, upg=upg, rb=rb, rcols=rcols, m0=m0,
        wcols=wcols, rwin=rwin, wwin=wwin, wpre=wpre, rtail=rtail, wtail=wtail,
        rows_per_ch=rows_per_ch)
    buf_bytes = nb * blk * S * TR * W * x.dtype.itemsize
    out = pl.pallas_call(
        kern,
        in_specs=[pl.BlockSpec(memory_space=pl.ANY)] * 3,
        out_specs=pl.BlockSpec(memory_space=pl.ANY),
        out_shape=jax.ShapeDtypeStruct(xr.shape, x.dtype),
        scratch_shapes=[
            pltpu.VMEM((nb, blk, S, TR, W), x.dtype),
            pltpu.VMEM((2, C // LANES, LANES), g.dtype),
            pltpu.VMEM((2, C, LANES), jnp.float32),
            pltpu.VMEM((3, nb * gpb, TR, rcols), jnp.float32),
            pltpu.VMEM((3, nb * gpb * cpg, LANES), jnp.float32),
            pltpu.SemaphoreType.DMA((2,)),
            pltpu.SemaphoreType.DMA((rwin,)),
            pltpu.SemaphoreType.DMA((wwin,)),
        ],
        compiler_params=pltpu.CompilerParams(
            vmem_limit_bytes=buf_bytes + 10 * 1024 * 1024,
            disable_bounds_checks=True,
            disable_semaphore_checks=True,
        ),
        interpret=interpret,
    )(g.reshape(C // LANES, LANES), b.reshape(C // LANES, LANES), xr)
    return out.reshape(B, C, H, W)


@jax.jit
def pallas_standalone__groupnorm__prompt_kernel(x, g, b):
    return _groupnorm(x, g, b)
```

```python
import functools

import jax
import jax.numpy as jnp
from jax import lax
import jax.experimental.pallas as pl
import jax.experimental.pallas.tpu as pltpu

NUM_GROUPS = 32
EPS = 1e-5

TR = 8
LANES = 128


def _div(i, n):
    if isinstance(i, int):
        return i // n
    if n & (n - 1) == 0:
        return lax.shift_right_logical(i, n.bit_length() - 1)
    return lax.div(i, n)


def _mod(i, n):
    if isinstance(i, int):
        return i % n
    if n & (n - 1) == 0:
        return lax.bitwise_and(i, n - 1)
    return lax.rem(i, n)


def _gn_kernel(g_hbm, b_hbm, x_hbm, o_hbm,
               buf, gb, gtab, part, coef, psem, rsem, wsem,
               *, rounds, upg, rb, rcols, m0, wcols, rwin, wwin, wpre, rtail,
               wtail, rows_per_ch):
    _, blk, S, _, W = x_hbm.shape
    nh = W // rcols
    rpb = S * nh
    gpb = blk // upg
    gpr = gpb * rb
    ch_per_unit = S // rows_per_ch
    cpb = blk * ch_per_unit
    cpg = upg * ch_per_unit
    n_ch = gtab.shape[1]
    n_pos = upg * rpb
    n_acc = TR * rcols
    wps = blk * S

    def rd_idx(t):
        r = _mod(t, rpb)
        c = _mod(r, nh) * rcols
        if not isinstance(c, int):
            c = pl.multiple_of(c, LANES)
        return _div(t, rpb) * rb, _div(r, nh), c

    def rd_start(base, t):
        b0, s, c = rd_idx(t)
        sem = rsem.at[_mod(t, rwin)]

        def cp(j, u0, n):
            return pltpu.make_async_copy(
                x_hbm.at[base + b0 + j, pl.ds(u0, n), s, :, pl.ds(c, rcols)],
                buf.at[b0 + j, pl.ds(u0, n), s, :, pl.ds(c, rcols)], sem)

        cp(0, m0, blk - m0).start(priority=1)
        for j in range(1, rb):
            cp(j, 0, blk).start(priority=1)
        cp(0, 0, m0).start(priority=0)

    def rd_wait(base, t):
        b0, s, c = rd_idx(t)
        pltpu.make_async_copy(
            x_hbm.at[pl.ds(base + b0, rb), :, s, :, pl.ds(c, rcols)],
            buf.at[pl.ds(b0, rb), :, s, :, pl.ds(c, rcols)],
            rsem.at[_mod(t, rwin)]).wait()

    def wr_start(base, b0, n, k, slot):
        u = _div(k, S)
        s = _mod(k, S)
        for c in range(0, W, wcols):
            pltpu.make_async_copy(
                buf.at[pl.ds(b0, n), u, s, :, pl.ds(c, wcols)],
                o_hbm.at[pl.ds(base + b0, n), u, s, :, pl.ds(c, wcols)],
                wsem.at[slot]).start()

    def wr_wait(base, b0, n, k, slot):
        u = _div(k, S)
        s = _mod(k, S)
        pltpu.make_async_copy(
            buf.at[pl.ds(b0, n), u, s], o_hbm.at[pl.ds(base + b0, n), u, s],
            wsem.at[slot]).wait()

    def rd_prologue(base):
        for t in range(rwin):
            rd_start(base, t)

    def load_chunk(t):
        b0, s, c = rd_idx(t)
        xb = buf[pl.ds(b0, rb), :, s, :, pl.ds(c, rcols)]
        return xb.astype(jnp.float32).reshape(gpr, upg, TR, rcols)

    def shifts(t):
        return load_chunk(t)[:, 0]

    def accumulate(t, ks, acc):
        d = load_chunk(t) - ks[:, None]
        return acc[0] + jnp.sum(d, axis=1), acc[1] + jnp.sum(d * d, axis=1)

    def save_partials(b0, ks, acc):
        for i, v in enumerate((ks,) + acc):
            part[i, pl.ds(b0 * gpb, gpr)] = v

    def finalize(base, b0, nb):
        g0, ng = b0 * gpb, nb * gpb
        k = part[0, g0:g0 + ng]
        s1 = part[1, g0:g0 + ng]
        s2 = part[2, g0:g0 + ng]
        d1 = s1 * (1.0 / n_pos)
        m = k + d1
        mean = jnp.sum(m, axis=(1, 2), keepdims=True) * (1.0 / n_acc)
        e = m - mean
        t = (s2 - s1 * d1) * (1.0 / n_pos) + e * e
        var = jnp.sum(t, axis=(1, 2), keepdims=True) * (1.0 / n_acc)
        rstd = lax.rsqrt(jnp.maximum(var, 0.0) + EPS)
        for i in range(ng):
            ch0 = ((base + b0) * gpb + i) * cpg % n_ch
            r0 = (g0 + i) * cpg
            coef[0, r0:r0 + cpg] = jnp.broadcast_to(mean[i], (cpg, LANES))
            coef[1, r0:r0 + cpg] = gtab[0, ch0:ch0 + cpg] * rstd[i]
            coef[2, r0:r0 + cpg] = gtab[1, ch0:ch0 + cpg]

    def normalize(b0, n, k):
        u = _div(k, S)
        s = _mod(k, S)
        row0 = _div(k, rows_per_ch)
        for j in range(n):
            cf = coef[:, pl.ds(row0 + (b0 + j) * cpb, 1), :]
            cf = jnp.tile(jnp.broadcast_to(cf, (3, TR, LANES)), (1, 1, W // LANES))
            xf = buf[b0 + j, u, s].astype(jnp.float32)
            buf[b0 + j, u, s] = ((xf - cf[0]) * cf[1] + cf[2]).astype(buf.dtype)

    zeros = (jnp.zeros((gpr, TR, rcols), jnp.float32),) * 2

    pcopies = [pltpu.make_async_copy(src, gb.at[i], psem.at[i])
               for i, src in enumerate((g_hbm, b_hbm))]
    for cp in pcopies:
        cp.start()
    rd_prologue(0)
    for cp in pcopies:
        cp.wait()
    for i in range(2):
        v = gb[i].astype(jnp.float32)
        for r in range(v.shape[0]):
            gtab[i, r * LANES:(r + 1) * LANES] = jnp.broadcast_to(
                v[r:r + 1, :], (LANES, LANES)).T

    base = 0
    for ri, sets in enumerate(rounds):
        nblk = sum(sets)
        nrb = nblk // rb
        nr = nrb * rpb
        last = ri + 1 == len(rounds)

        rd_wait(base, 0)
        rd_start(base, rwin)

        def rd_body(t, ks, acc, base=base):
            acc = accumulate(t, ks, acc)
            rd_wait(base, t + 1)
            rd_start(base, t + 1 + rwin)
            return acc

        def blk_body(bi, carry, rd_body=rd_body):
            ks = shifts(bi * rpb)
            acc = lax.fori_loop(
                0, rpb, lambda r, acc: rd_body(bi * rpb + r, ks, acc), zeros)
            save_partials(bi * rb, ks, acc)
            return carry

        lax.fori_loop(0, nrb - 1, blk_body, 0)
        ks = shifts(nr - rpb)
        acc = lax.fori_loop(
            nr - rpb, nr - rwin - 1, lambda t, acc: rd_body(t, ks, acc), zeros)

        n0 = sets[0]
        finalize(base, 0, n0)
        for k in range(wpre):
            normalize(0, n0, k)
        for t in range(nr - rwin, nr - rtail):
            rd_wait(base, t)
        for k in range(wpre):
            wr_start(base, 0, n0, k, k)

        def wr_fill(k, carry, base=base, n0=n0):
            normalize(0, n0, k)
            wr_start(base, 0, n0, k, k)
            return carry

        lax.fori_loop(wpre, wwin, wr_fill, 0)
        for t in range(nr - rtail, nr):
            rd_wait(base, t)
        acc = lax.fori_loop(
            nr - rwin - 1, nr, lambda t, acc: accumulate(t, ks, acc), acc)
        save_partials(nblk - rb, ks, acc)
        finalize(base, n0, nblk - n0)

        b0 = 0
        for si, n in enumerate(sets):
            if si > 0:
                def wr_edge(k, carry, base=base, b0=b0, n=n, np_=sets[si - 1]):
                    normalize(b0, n, k)
                    wr_wait(base, b0 - np_, np_, wps - wwin + k, k)
                    wr_start(base, b0, n, k, k)
                    return carry

                lax.fori_loop(0, wwin, wr_edge, 0)

            def wr_body(k, carry, base=base, b0=b0, n=n):
                slot = _mod(k, wwin)
                normalize(b0, n, k)
                wr_wait(base, b0, n, k - wwin, slot)
                wr_start(base, b0, n, k, slot)
                return carry

            lax.fori_loop(wwin, wps, wr_body, 0)
            b0 += n

        n = sets[-1]
        for k in range(wps - wwin, wps + 1):
            if k == wps - wtail and not last:
                rd_prologue(base + nblk)
            if k < wps:
                wr_wait(base, nblk - n, n, k, k % wwin)
        base += nblk


def _groupnorm(x, g, b, *, S=32, blk=8, rb=2, rcols=256, m0=2, wcols=256,
               rwin=16, wwin=16, wpre=2, rtail=8, wtail=1,
               rounds=((6, 6), (5, 5), (5, 5)), interpret=False):
    B, C, H, W = x.shape
    G = NUM_GROUPS
    cpg = C // G
    rows_per_ch = H // TR
    assert H % TR == 0 and S % rows_per_ch == 0
    assert W % rcols == 0 and W % wcols == 0 and C % LANES == 0
    tr_per_group = cpg * rows_per_ch
    assert tr_per_group % S == 0
    upg = tr_per_group // S
    A = B * G * upg
    assert blk % upg == 0 and A % blk == 0
    nblk = A // blk
    assert sum(sum(r) for r in rounds) == nblk
    for r in rounds:
        assert sum(r) % rb == 0 and len(r) >= 2 and rb <= r[0] <= sum(r) - rb
    assert wpre <= wwin and (blk * S) % wwin == 0 and wtail <= wwin
    assert rtail <= rwin < S * (W // rcols) and 0 < m0 < blk
    nb = max(sum(r) for r in rounds)
    gpb = blk // upg
    xr = x.reshape(nblk, blk, S, TR, W)
    kern = functools.partial(
        _gn_kernel, rounds=rounds, upg=upg, rb=rb, rcols=rcols, m0=m0,
        wcols=wcols, rwin=rwin, wwin=wwin, wpre=wpre, rtail=rtail, wtail=wtail,
        rows_per_ch=rows_per_ch)
    buf_bytes = nb * blk * S * TR * W * x.dtype.itemsize
    opts = {name: True
            for name in ("disable_bounds_checks", "disable_semaphore_checks")
            if hasattr(pltpu.CompilerParams, name)}
    out = pl.pallas_call(
        kern,
        in_specs=[pl.BlockSpec(memory_space=pl.ANY)] * 3,
        out_specs=pl.BlockSpec(memory_space=pl.ANY),
        out_shape=jax.ShapeDtypeStruct(xr.shape, x.dtype),
        scratch_shapes=[
            pltpu.VMEM((nb, blk, S, TR, W), x.dtype),
            pltpu.VMEM((2, C // LANES, LANES), g.dtype),
            pltpu.VMEM((2, C, LANES), jnp.float32),
            pltpu.VMEM((3, nb * gpb, TR, rcols), jnp.float32),
            pltpu.VMEM((3, nb * gpb * cpg, LANES), jnp.float32),
            pltpu.SemaphoreType.DMA((2,)),
            pltpu.SemaphoreType.DMA((rwin,)),
            pltpu.SemaphoreType.DMA((wwin,)),
        ],
        compiler_params=pltpu.CompilerParams(
            vmem_limit_bytes=buf_bytes + 10 * 1024 * 1024, **opts),
        interpret=interpret,
    )(g.reshape(C // LANES, LANES), b.reshape(C // LANES, LANES), xr)
    return out.reshape(B, C, H, W)


@jax.jit
def pallas_standalone__groupnorm__prompt_kernel(x, g, b):
    return _groupnorm(x, g, b)
```

```python
import functools

import jax
import jax.numpy as jnp
from jax import lax
import jax.experimental.pallas as pl
import jax.experimental.pallas.tpu as pltpu

NUM_GROUPS = 32
EPS = 1e-5

TR = 8
LANES = 128


def _div(i, n):
    if isinstance(i, int):
        return i // n
    if n & (n - 1) == 0:
        return lax.shift_right_logical(i, n.bit_length() - 1)
    return lax.div(i, n)


def _mod(i, n):
    if isinstance(i, int):
        return i % n
    if n & (n - 1) == 0:
        return lax.bitwise_and(i, n - 1)
    return lax.rem(i, n)


def _gn_kernel(g_hbm, b_hbm, x_hbm, o_hbm,
               buf, gb, gtab, part, coef, psem, rsem, wsem,
               *, rounds, upg, rb, rcols, m0, wcols, rwin, wwin, wpre, rtail,
               wtail, rows_per_ch):
    _, blk, S, _, W = x_hbm.shape
    nh = W // rcols
    rpb = S * nh
    gpb = blk // upg
    ch_per_unit = S // rows_per_ch
    cpb = blk * ch_per_unit
    cpg = upg * ch_per_unit
    n_ch = gtab.shape[1]
    n_pos = upg * rpb
    n_acc = TR * rcols
    wps = blk * S

    def rd_idx(t):
        r = _mod(t, rpb)
        c = _mod(r, nh) * rcols
        if not isinstance(c, int):
            c = pl.multiple_of(c, LANES)
        return _div(t, rpb) * rb, _div(r, nh), c

    def rd_start(base, t):
        b0, s, c = rd_idx(t)
        sem = rsem.at[_mod(t, rwin)]

        def cp(j, u0, n):
            return pltpu.make_async_copy(
                x_hbm.at[base + b0 + j, pl.ds(u0, n), s, :, pl.ds(c, rcols)],
                buf.at[b0 + j, pl.ds(u0, n), s, :, pl.ds(c, rcols)], sem)

        cp(0, m0, blk - m0).start(priority=1)
        for j in range(1, rb):
            cp(j, 0, blk).start(priority=1)
        cp(0, 0, m0).start(priority=0)

    def rd_wait(base, t):
        b0, s, c = rd_idx(t)
        pltpu.make_async_copy(
            x_hbm.at[pl.ds(base + b0, rb), :, s, :, pl.ds(c, rcols)],
            buf.at[pl.ds(b0, rb), :, s, :, pl.ds(c, rcols)],
            rsem.at[_mod(t, rwin)]).wait()

    def wr_start(base, b0, n, k, slot):
        u = _div(k, S)
        s = _mod(k, S)
        for c in range(0, W, wcols):
            pltpu.make_async_copy(
                buf.at[pl.ds(b0, n), u, s, :, pl.ds(c, wcols)],
                o_hbm.at[pl.ds(base + b0, n), u, s, :, pl.ds(c, wcols)],
                wsem.at[slot]).start()

    def wr_wait(base, b0, n, k, slot):
        u = _div(k, S)
        s = _mod(k, S)
        pltpu.make_async_copy(
            buf.at[pl.ds(b0, n), u, s], o_hbm.at[pl.ds(base + b0, n), u, s],
            wsem.at[slot]).wait()

    def rd_prologue(base):
        for t in range(rwin):
            rd_start(base, t)

    def load_chunk(t):
        b0, s, c = rd_idx(t)
        return [buf[b0 + j, :, s, :, pl.ds(c, rcols)] for j in range(rb)]

    def widen(xb):
        return xb.astype(jnp.float32).reshape(gpb, upg, TR, rcols)

    def shifts(t):
        return tuple(widen(xb)[:, 0] for xb in load_chunk(t))

    def accumulate(xs, ks, acc):
        out = []
        for j in range(rb):
            d = widen(xs[j]) - ks[j][:, None]
            out.append(acc[2 * j] + jnp.sum(d, axis=1))
            out.append(acc[2 * j + 1] + jnp.sum(d * d, axis=1))
        return tuple(out)

    def save_partials(b0, ks, acc):
        for j in range(rb):
            rows = pl.ds((b0 + j) * gpb, gpb)
            part[0, rows] = ks[j]
            part[1, rows] = acc[2 * j]
            part[2, rows] = acc[2 * j + 1]

    def finalize(base, b0, nb):
        g0, ng = b0 * gpb, nb * gpb
        k = part[0, g0:g0 + ng]
        s1 = part[1, g0:g0 + ng]
        s2 = part[2, g0:g0 + ng]
        d1 = s1 * (1.0 / n_pos)
        m = k + d1
        mean = jnp.sum(m, axis=(1, 2), keepdims=True) * (1.0 / n_acc)
        e = m - mean
        t = (s2 - s1 * d1) * (1.0 / n_pos) + e * e
        var = jnp.sum(t, axis=(1, 2), keepdims=True) * (1.0 / n_acc)
        rstd = lax.rsqrt(jnp.maximum(var, 0.0) + EPS)
        for i in range(ng):
            ch0 = ((base + b0) * gpb + i) * cpg % n_ch
            r0 = (g0 + i) * cpg
            coef[0, r0:r0 + cpg] = jnp.broadcast_to(mean[i], (cpg, LANES))
            coef[1, r0:r0 + cpg] = gtab[0, ch0:ch0 + cpg] * rstd[i]
            coef[2, r0:r0 + cpg] = gtab[1, ch0:ch0 + cpg]

    def normalize(b0, n, k):
        u = _div(k, S)
        s = _mod(k, S)
        row0 = _div(k, rows_per_ch)
        for j in range(n):
            cf = coef[:, pl.ds(row0 + (b0 + j) * cpb, 1), :]
            cf = jnp.tile(jnp.broadcast_to(cf, (3, TR, LANES)), (1, 1, W // LANES))
            xf = buf[b0 + j, u, s].astype(jnp.float32)
            buf[b0 + j, u, s] = ((xf - cf[0]) * cf[1] + cf[2]).astype(buf.dtype)

    zeros = (jnp.zeros((gpb, TR, rcols), jnp.float32),) * (2 * rb)

    pcopies = [pltpu.make_async_copy(src, gb.at[i], psem.at[i])
               for i, src in enumerate((g_hbm, b_hbm))]
    for cp in pcopies:
        cp.start()
    rd_prologue(0)
    for cp in pcopies:
        cp.wait()
    for i in range(2):
        v = gb[i].astype(jnp.float32)
        for r in range(v.shape[0]):
            gtab[i, r * LANES:(r + 1) * LANES] = jnp.broadcast_to(
                v[r:r + 1, :], (LANES, LANES)).T

    base = 0
    for ri, sets in enumerate(rounds):
        nblk = sum(sets)
        nrb = nblk // rb
        nr = nrb * rpb
        last = ri + 1 == len(rounds)

        rd_wait(base, 0)
        rd_start(base, rwin)

        def rd_body(t, ks, acc, base=base):
            xs = load_chunk(t)
            rd_wait(base, t + 1)
            rd_start(base, t + 1 + rwin)
            return accumulate(xs, ks, acc)

        def blk_body(bi, carry, rd_body=rd_body):
            ks = shifts(bi * rpb)
            acc = lax.fori_loop(
                0, rpb, lambda r, acc: rd_body(bi * rpb + r, ks, acc), zeros)
            save_partials(bi * rb, ks, acc)
            return carry

        lax.fori_loop(0, nrb - 1, blk_body, 0)
        ks = shifts(nr - rpb)
        acc = lax.fori_loop(
            nr - rpb, nr - rwin - 1, lambda t, acc: rd_body(t, ks, acc), zeros)

        n0 = sets[0]
        finalize(base, 0, n0)
        for k in range(wpre):
            normalize(0, n0, k)
        for t in range(nr - rwin, nr - rtail):
            rd_wait(base, t)
        for k in range(wpre):
            wr_start(base, 0, n0, k, k)

        def wr_fill(k, carry, base=base, n0=n0):
            normalize(0, n0, k)
            wr_start(base, 0, n0, k, k)
            return carry

        lax.fori_loop(wpre, wwin, wr_fill, 0)
        for t in range(nr - rtail, nr):
            rd_wait(base, t)
        acc = lax.fori_loop(
            nr - rwin - 1, nr, lambda t, acc: accumulate(load_chunk(t), ks, acc), acc)
        save_partials(nblk - rb, ks, acc)
        finalize(base, n0, nblk - n0)

        b0 = 0
        for si, n in enumerate(sets):
            if si > 0:
                def wr_edge(k, carry, base=base, b0=b0, n=n, np_=sets[si - 1]):
                    normalize(b0, n, k)
                    wr_wait(base, b0 - np_, np_, wps - wwin + k, k)
                    wr_start(base, b0, n, k, k)
                    return carry

                lax.fori_loop(0, wwin, wr_edge, 0)

            def wr_body(k, carry, base=base, b0=b0, n=n):
                slot = _mod(k, wwin)
                normalize(b0, n, k)
                wr_wait(base, b0, n, k - wwin, slot)
                wr_start(base, b0, n, k, slot)
                return carry

            lax.fori_loop(wwin, wps, wr_body, 0)
            b0 += n

        n = sets[-1]
        for k in range(wps - wwin, wps + 1):
            if k == wps - wtail and not last:
                rd_prologue(base + nblk)
            if k < wps:
                wr_wait(base, nblk - n, n, k, k % wwin)
        base += nblk


def _groupnorm(x, g, b, *, S=32, blk=8, rb=2, rcols=256, m0=2, wcols=256,
               rwin=16, wwin=16, wpre=3, rtail=8, wtail=0,
               rounds=((6, 6), (5, 5), (5, 5)), checks=False, interpret=False):
    B, C, H, W = x.shape
    G = NUM_GROUPS
    cpg = C // G
    rows_per_ch = H // TR
    assert H % TR == 0 and S % rows_per_ch == 0
    assert W % rcols == 0 and W % wcols == 0 and C % LANES == 0
    tr_per_group = cpg * rows_per_ch
    assert tr_per_group % S == 0
    upg = tr_per_group // S
    A = B * G * upg
    assert blk % upg == 0 and A % blk == 0
    nblk = A // blk
    assert sum(sum(r) for r in rounds) == nblk
    for r in rounds:
        assert sum(r) % rb == 0 and len(r) >= 2 and rb <= r[0] <= sum(r) - rb
    assert wpre <= wwin and (blk * S) % wwin == 0 and wtail <= wwin
    assert rtail <= rwin < S * (W // rcols) and 0 < m0 < blk
    nb = max(sum(r) for r in rounds)
    gpb = blk // upg
    xr = x.reshape(nblk, blk, S, TR, W)
    kern = functools.partial(
        _gn_kernel, rounds=rounds, upg=upg, rb=rb, rcols=rcols, m0=m0,
        wcols=wcols, rwin=rwin, wwin=wwin, wpre=wpre, rtail=rtail, wtail=wtail,
        rows_per_ch=rows_per_ch)
    buf_bytes = nb * blk * S * TR * W * x.dtype.itemsize
    opts = {name: not checks
            for name in ("disable_bounds_checks", "disable_semaphore_checks")
            if hasattr(pltpu.CompilerParams, name)}
    out = pl.pallas_call(
        kern,
        in_specs=[pl.BlockSpec(memory_space=pl.ANY)] * 3,
        out_specs=pl.BlockSpec(memory_space=pl.ANY),
        out_shape=jax.ShapeDtypeStruct(xr.shape, x.dtype),
        scratch_shapes=[
            pltpu.VMEM((nb, blk, S, TR, W), x.dtype),
            pltpu.VMEM((2, C // LANES, LANES), g.dtype),
            pltpu.VMEM((2, C, LANES), jnp.float32),
            pltpu.VMEM((3, nb * gpb, TR, rcols), jnp.float32),
            pltpu.VMEM((3, nb * gpb * cpg, LANES), jnp.float32),
            pltpu.SemaphoreType.DMA((2,)),
            pltpu.SemaphoreType.DMA((rwin,)),
            pltpu.SemaphoreType.DMA((wwin,)),
        ],
        compiler_params=pltpu.CompilerParams(
            vmem_limit_bytes=buf_bytes + 10 * 1024 * 1024, **opts),
        interpret=interpret,
    )(g.reshape(C // LANES, LANES), b.reshape(C // LANES, LANES), xr)
    return out.reshape(B, C, H, W)


@jax.jit
def pallas_standalone__groupnorm__prompt_kernel(x, g, b):
    return _groupnorm(x, g, b)
```

```python
import functools

import jax
import jax.numpy as jnp
from jax import lax
import jax.experimental.pallas as pl
import jax.experimental.pallas.tpu as pltpu

NUM_GROUPS = 32
EPS = 1e-5

TR = 8
LANES = 128


def _div(i, n):
    if isinstance(i, int):
        return i // n
    if n & (n - 1) == 0:
        return lax.shift_right_logical(i, n.bit_length() - 1)
    return lax.div(i, n)


def _mod(i, n):
    if isinstance(i, int):
        return i % n
    if n & (n - 1) == 0:
        return lax.bitwise_and(i, n - 1)
    return lax.rem(i, n)


def _gn_kernel(g_hbm, b_hbm, x_hbm, o_hbm,
               buf, gb, gtab, part, coef, psem, rsem, wsem,
               *, rounds, upg, rb, rcols, m0, wcols, rwin, wwin, wpre, rtail,
               wtail, rows_per_ch):
    _, blk, S, _, W = x_hbm.shape
    nh = W // rcols
    rpb = S * nh
    gpb = blk // upg
    ch_per_unit = S // rows_per_ch
    cpg = upg * ch_per_unit
    n_ch = gtab.shape[1]
    n_pos = upg * rpb
    n_acc = TR * rcols
    wps = blk * S

    def rd_idx(t):
        r = _mod(t, rpb)
        c = _mod(r, nh) * rcols
        if not isinstance(c, int):
            c = pl.multiple_of(c, LANES)
        return _div(t, rpb) * rb, _div(r, nh), c

    def rd_start(base, t):
        b0, s, c = rd_idx(t)
        sem = rsem.at[_mod(t, rwin)]

        def cp(j, u0, n):
            return pltpu.make_async_copy(
                x_hbm.at[base + b0 + j, pl.ds(u0, n), s, :, pl.ds(c, rcols)],
                buf.at[b0 + j, pl.ds(u0, n), s, :, pl.ds(c, rcols)], sem)

        cp(0, m0, blk - m0).start(priority=1)
        for j in range(1, rb):
            cp(j, 0, blk).start(priority=1)
        cp(0, 0, m0).start(priority=0)

    def rd_wait(base, t):
        b0, s, c = rd_idx(t)
        pltpu.make_async_copy(
            x_hbm.at[pl.ds(base + b0, rb), :, s, :, pl.ds(c, rcols)],
            buf.at[pl.ds(b0, rb), :, s, :, pl.ds(c, rcols)],
            rsem.at[_mod(t, rwin)]).wait()

    def wr_start(base, b0, n, k, slot):
        u = _div(k, S)
        s = _mod(k, S)
        for c in range(0, W, wcols):
            pltpu.make_async_copy(
                buf.at[pl.ds(b0, n), u, s, :, pl.ds(c, wcols)],
                o_hbm.at[pl.ds(base + b0, n), u, s, :, pl.ds(c, wcols)],
                wsem.at[slot]).start()

    def wr_wait(base, b0, n, k, slot):
        u = _div(k, S)
        s = _mod(k, S)
        pltpu.make_async_copy(
            buf.at[pl.ds(b0, n), u, s], o_hbm.at[pl.ds(base + b0, n), u, s],
            wsem.at[slot]).wait()

    def rd_prologue(base):
        for t in range(rwin):
            rd_start(base, t)

    def load_chunk(t):
        b0, s, c = rd_idx(t)
        return [buf[b0 + j, :, s, :, pl.ds(c, rcols)] for j in range(rb)]

    def widen(xb):
        return xb.astype(jnp.float32).reshape(gpb, upg, TR, rcols)

    def shifts(t):
        return tuple(widen(xb)[:, 0] for xb in load_chunk(t))

    def accumulate(xs, ks, acc):
        out = []
        for j in range(rb):
            d = widen(xs[j]) - ks[j][:, None]
            out.append(acc[2 * j] + jnp.sum(d, axis=1))
            out.append(acc[2 * j + 1] + jnp.sum(d * d, axis=1))
        return tuple(out)

    def save_partials(b0, ks, acc):
        for j in range(rb):
            rows = pl.ds((b0 + j) * gpb, gpb)
            part[0, rows] = ks[j]
            part[1, rows] = acc[2 * j]
            part[2, rows] = acc[2 * j + 1]

    def finalize(base, b0, nb):
        g0, ng = b0 * gpb, nb * gpb
        k = part[0, g0:g0 + ng]
        s1 = part[1, g0:g0 + ng]
        s2 = part[2, g0:g0 + ng]
        d1 = s1 * (1.0 / n_pos)
        m = k + d1
        mean = jnp.sum(m, axis=(1, 2), keepdims=True) * (1.0 / n_acc)
        e = m - mean
        t = (s2 - s1 * d1) * (1.0 / n_pos) + e * e
        var = jnp.sum(t, axis=(1, 2), keepdims=True) * (1.0 / n_acc)
        rstd = lax.rsqrt(jnp.maximum(var, 0.0) + EPS)
        for i in range(ng):
            ch0 = ((base + b0) * gpb + i) * cpg % n_ch
            bi, r0 = b0 + i // gpb, (i % gpb) * cpg
            coef[0, bi, r0:r0 + cpg] = jnp.broadcast_to(mean[i], (cpg, LANES))
            coef[1, bi, r0:r0 + cpg] = gtab[0, ch0:ch0 + cpg] * rstd[i]
            coef[2, bi, r0:r0 + cpg] = gtab[1, ch0:ch0 + cpg]

    def normalize(b0, n, k):
        u = _div(k, S)
        s = _mod(k, S)
        row = _div(k, rows_per_ch)
        mean, scale, bias = (
            jnp.tile(jnp.broadcast_to(coef[i, b0:b0 + n, pl.ds(row, 1), :],
                                      (n, TR, LANES)), (1, 1, W // LANES))
            for i in range(3))
        xf = buf[b0:b0 + n, u, s].astype(jnp.float32)
        buf[b0:b0 + n, u, s] = ((xf - mean) * scale + bias).astype(buf.dtype)

    zeros = (jnp.zeros((gpb, TR, rcols), jnp.float32),) * (2 * rb)

    pcopies = [pltpu.make_async_copy(src, gb.at[i], psem.at[i])
               for i, src in enumerate((g_hbm, b_hbm))]
    for cp in pcopies:
        cp.start()
    rd_prologue(0)
    for cp in pcopies:
        cp.wait()
    for i in range(2):
        v = gb[i].astype(jnp.float32)
        for r in range(v.shape[0]):
            gtab[i, r * LANES:(r + 1) * LANES] = jnp.broadcast_to(
                v[r:r + 1, :], (LANES, LANES)).T

    base = 0
    for ri, sets in enumerate(rounds):
        nblk = sum(sets)
        nrb = nblk // rb
        nr = nrb * rpb
        last = ri + 1 == len(rounds)

        rd_wait(base, 0)
        rd_start(base, rwin)

        def rd_body(t, ks, acc, base=base):
            xs = load_chunk(t)
            rd_wait(base, t + 1)
            rd_start(base, t + 1 + rwin)
            return accumulate(xs, ks, acc)

        def blk_body(bi, carry, rd_body=rd_body):
            ks = shifts(bi * rpb)
            acc = lax.fori_loop(
                0, rpb, lambda r, acc: rd_body(bi * rpb + r, ks, acc), zeros)
            save_partials(bi * rb, ks, acc)
            return carry

        lax.fori_loop(0, nrb - 1, blk_body, 0)
        ks = shifts(nr - rpb)
        acc = lax.fori_loop(
            nr - rpb, nr - rwin - 1, lambda t, acc: rd_body(t, ks, acc), zeros)

        n0 = sets[0]
        finalize(base, 0, n0)
        for k in range(wpre):
            normalize(0, n0, k)
        for t in range(nr - rwin, nr - rtail):
            rd_wait(base, t)
        for k in range(wpre):
            wr_start(base, 0, n0, k, k)

        def wr_fill(k, carry, base=base, n0=n0):
            normalize(0, n0, k)
            wr_start(base, 0, n0, k, k)
            return carry

        lax.fori_loop(wpre, wwin, wr_fill, 0)
        for t in range(nr - rtail, nr):
            rd_wait(base, t)
        acc = lax.fori_loop(
            nr - rwin - 1, nr, lambda t, acc: accumulate(load_chunk(t), ks, acc), acc)
        save_partials(nblk - rb, ks, acc)
        finalize(base, n0, nblk - n0)

        b0 = 0
        for si, n in enumerate(sets):
            if si > 0:
                def wr_edge(k, carry, base=base, b0=b0, n=n, np_=sets[si - 1]):
                    normalize(b0, n, k)
                    wr_wait(base, b0 - np_, np_, wps - wwin + k, k)
                    wr_start(base, b0, n, k, k)
                    return carry

                lax.fori_loop(0, wwin, wr_edge, 0)

            def wr_body(k, carry, base=base, b0=b0, n=n):
                slot = _mod(k, wwin)
                normalize(b0, n, k)
                wr_wait(base, b0, n, k - wwin, slot)
                wr_start(base, b0, n, k, slot)
                return carry

            lax.fori_loop(wwin, wps, wr_body, 0)
            b0 += n

        n = sets[-1]
        for k in range(wps - wwin, wps + 1):
            if k == wps - wtail and not last:
                rd_prologue(base + nblk)
            if k < wps:
                wr_wait(base, nblk - n, n, k, k % wwin)
        base += nblk


def _groupnorm(x, g, b, *, S=32, blk=8, rb=2, rcols=256, m0=2, wcols=256,
               rwin=16, wwin=16, wpre=3, rtail=8, wtail=0,
               rounds=((6, 6), (5, 5), (5, 5)), checks=False, interpret=False):
    B, C, H, W = x.shape
    G = NUM_GROUPS
    cpg = C // G
    rows_per_ch = H // TR
    assert H % TR == 0 and S % rows_per_ch == 0
    assert W % rcols == 0 and W % wcols == 0 and C % LANES == 0
    tr_per_group = cpg * rows_per_ch
    assert tr_per_group % S == 0
    upg = tr_per_group // S
    A = B * G * upg
    assert blk % upg == 0 and A % blk == 0
    nblk = A // blk
    assert sum(sum(r) for r in rounds) == nblk
    for r in rounds:
        assert sum(r) % rb == 0 and len(r) >= 2 and rb <= r[0] <= sum(r) - rb
    assert wpre <= wwin and (blk * S) % wwin == 0 and wtail <= wwin
    assert rtail <= rwin < S * (W // rcols) and 0 < m0 < blk
    nb = max(sum(r) for r in rounds)
    gpb = blk // upg
    xr = x.reshape(nblk, blk, S, TR, W)
    kern = functools.partial(
        _gn_kernel, rounds=rounds, upg=upg, rb=rb, rcols=rcols, m0=m0,
        wcols=wcols, rwin=rwin, wwin=wwin, wpre=wpre, rtail=rtail, wtail=wtail,
        rows_per_ch=rows_per_ch)
    buf_bytes = nb * blk * S * TR * W * x.dtype.itemsize
    opts = {name: not checks
            for name in ("disable_bounds_checks", "disable_semaphore_checks")
            if hasattr(pltpu.CompilerParams, name)}
    out = pl.pallas_call(
        kern,
        in_specs=[pl.BlockSpec(memory_space=pl.ANY)] * 3,
        out_specs=pl.BlockSpec(memory_space=pl.ANY),
        out_shape=jax.ShapeDtypeStruct(xr.shape, x.dtype),
        scratch_shapes=[
            pltpu.VMEM((nb, blk, S, TR, W), x.dtype),
            pltpu.VMEM((2, C // LANES, LANES), g.dtype),
            pltpu.VMEM((2, C, LANES), jnp.float32),
            pltpu.VMEM((3, nb * gpb, TR, rcols), jnp.float32),
            pltpu.VMEM((3, nb, gpb * cpg, LANES), jnp.float32),
            pltpu.SemaphoreType.DMA((2,)),
            pltpu.SemaphoreType.DMA((rwin,)),
            pltpu.SemaphoreType.DMA((wwin,)),
        ],
        compiler_params=pltpu.CompilerParams(
            vmem_limit_bytes=buf_bytes + 10 * 1024 * 1024, **opts),
        interpret=interpret,
    )(g.reshape(C // LANES, LANES), b.reshape(C // LANES, LANES), xr)
    return out.reshape(B, C, H, W)


@jax.jit
def pallas_standalone__groupnorm__prompt_kernel(x, g, b):
    return _groupnorm(x, g, b)
```
